```python
import os as _os
_os.environ.setdefault("JAX_PLATFORMS", "cpu")
import jax
import jax.numpy as jnp

def _softmax(x, axis=-1):
    return jax.nn.softmax(x, axis=axis)
def _gelu(x):
    return jax.nn.gelu(x, approximate=True)
def _silu(x):
    return jax.nn.silu(x)
def _sigmoid(x):
    return jax.nn.sigmoid(x)
def _layernorm(x, axis=-1, eps=1e-5):
    m = jnp.mean(x, axis=axis, keepdims=True)
    v = jnp.var(x, axis=axis, keepdims=True)
    return (x - m) / jnp.sqrt(v + eps)
def _scatter_add(tgt, idx, src, axis=0):
    return tgt.at[idx].add(src)
def _segment_sum(src, seg, n):
    return jax.ops.segment_sum(src, seg, n)
class _Rng:
    def __init__(self, key):
        self._k = key
    def _next(self):
        self._k, sub = jax.random.split(self._k)
        return sub
    def normal(self, shape):
        return jax.random.normal(self._next(), shape, dtype=jnp.bfloat16)
    def randint(self, lo, hi, shape):
        return jax.random.randint(self._next(), shape, lo, hi, dtype=jnp.int32)
    def uniform(self, shape, lo=0.0, hi=1.0):
        return jax.random.uniform(self._next(), shape, jnp.bfloat16, lo, hi)
    def permutation(self, n):
        return jax.random.permutation(self._next(), n)


kernel_name = 'parallel_sum__mha_block__swiglu_ffn__prompt'

def setup_inputs():
    _rng = _Rng(jax.random.key(int.from_bytes(__import__("os").urandom(4), "little")))
    _w = (lambda a: (lambda t: t.astype(jnp.bfloat16) if jnp.issubdtype(t.dtype, jnp.floating) else t)(jnp.asarray(a)))
    def _A_setup():
        B, S, D, H = 1, 2048, 512, 32
        return {
            "x": _w((lambda *s: _rng.normal(s) * 0.05)(B, S, D)),
            "wqkv": _w((lambda *s: _rng.normal(s) * 0.1)(D, 3 * D)),
            "wo": _w((lambda *s: _rng.normal(s) * 0.05)(D, D)),
        }
    _A_in = _A_setup()

    def _B_setup():
        B, S, D, F = 1, 2048, 512, 1792
        return {
            "x": _w((lambda *s: _rng.normal(s) * 0.05)(B, S, D)),
            "w_gate": _w((lambda *s: _rng.normal(s) * 0.05)(D, F)),
            "w_up": _w((lambda *s: _rng.normal(s) * 0.05)(D, F)),
            "w_down": _w((lambda *s: _rng.normal(s) * 0.05)(F, D)),
        }
    _B_in = _B_setup()

    return {
        "A_x": _A_in["x"],
        "A_wqkv": _A_in["wqkv"],
        "A_wo": _A_in["wo"],
        "B_x": _B_in["x"],
        "B_w_gate": _B_in["w_gate"],
        "B_w_up": _B_in["w_up"],
        "B_w_down": _B_in["w_down"],
    }

def reference(A_x, A_wqkv, A_wo, B_x, B_w_gate, B_w_up, B_w_down):
    def _A_ref(x, wqkv, wo):
        B, S, D = x.shape
        H = 32
        Dh = D // H
        qkv = (lambda x, *d: x.transpose(*d))((x @ wqkv).reshape(B, S, 3, H, Dh), 2, 0, 3, 1, 4)
        q, k, v = qkv[0], qkv[1], qkv[2]
        scores = jnp.einsum("bhqd,bhkd->bhqk", q, k) * (Dh ** -0.5)
        p = _softmax(scores, axis=-1)
        o = jnp.einsum("bhqk,bhkd->bhqd", p, v)
        return (lambda x, *d: x.transpose(*d))(o, 0, 2, 1, 3).reshape(B, S, D) @ wo

    def _B_ref(x, w_gate, w_up, w_down):
        g = _silu(x @ w_gate)
        u = x @ w_up
        return (g * u) @ w_down

    x = A_x
    xn = _layernorm(x, axis=-1)
    return x + _A_ref(xn, A_wqkv, A_wo) + _B_ref(xn, B_w_gate, B_w_up, B_w_down)
```

```python
import jax
import jax.numpy as jnp
import jax.experimental.pallas as pl
import jax.experimental.pallas.tpu as pltpu

S, D, H, DH, F = 2048, 512, 32, 16, 1792
TQ = 512
TM = 256
CK = 128
U = 8
SK = 2
BIG = 2.0 ** 100
TL = 128
LOG2E = 1.4426950408889634
bf = jnp.bfloat16
f32 = jnp.float32
NT = (((1,), (1,)), ((), ()))


def _kernel(x_h, wqkv_h, wo_h, wg_h, wu_h, wd_h, o_h,
            x_ref, wqkv_ref, wo_ref, wg_ref, wu_ref, wd_ref, o_ref, sems, xn_s, qT_s, k_s, vT_s, oT_s, wT_s):
    NB = S // TM
    cps = [pltpu.make_async_copy(wqkv_h, wqkv_ref, sems.at[0])]
    cps += [pltpu.make_async_copy(a, b, sems.at[1 + n]) for n, (a, b) in enumerate(
        [(wg_h, wg_ref), (wu_h, wu_ref), (wd_h, wd_ref), (wo_h, wo_ref)])]

    def xcp(i):
        r = pl.ds(pl.multiple_of(i * TM, TM), TM)
        return pltpu.make_async_copy(x_h.at[r, :], x_ref.at[r, :], sems.at[5 + i])

    def ocp(i):
        r = pl.ds(pl.multiple_of(i * TM, TM), TM)
        return pltpu.make_async_copy(o_ref.at[r, :], o_h.at[r, :], sems.at[5 + NB + i])
    xcp(0).start()
    cps[0].start()
    for i in range(1, NB):
        xcp(i).start()
    for cp in cps[1:]:
        cp.start()

    def ln(i):
        xcp(i).wait()
        r = pl.ds(pl.multiple_of(i * TM, TM), TM)
        x = x_ref[r, :].astype(f32)
        m = jnp.mean(x, axis=-1, keepdims=True)
        xc = x - m
        v = jnp.mean(xc * xc, axis=-1, keepdims=True)
        xn_s[r, :] = (xc * jax.lax.rsqrt(v + 1e-5)).astype(bf)

    def proj(i):
        r = pl.ds(pl.multiple_of(i * TM, TM), TM)
        xn = xn_s[r, :]
        k_s[r, :] = jnp.dot(xn, wqkv_ref[:, D:2 * D], preferred_element_type=f32).astype(bf)
        q = jax.lax.dot_general(wT_s[0], xn, NT, preferred_element_type=f32)
        qT_s[:, r] = (q * (DH ** -0.5 * LOG2E)).astype(bf)
        vT_s[:, r] = jax.lax.dot_general(wT_s[1], xn, NT, preferred_element_type=f32).astype(bf)

    ln(0)
    cps[0].wait()
    wT_s[0] = wqkv_ref[:, :D].T
    wT_s[1] = wqkv_ref[:, 2 * D:].T
    for i in range(NB):
        if i + 1 < NB:
            ln(i + 1)
        proj(i)

    NQ = S // TQ
    NC = S // CK
    row = jax.lax.broadcasted_iota(jnp.int32, (128, TQ), 0)

    def getq(i):
        h = i // NQ
        qt = i % NQ
        gs = pl.ds(pl.multiple_of((h // 8) * 128, 128), 128)
        qs = pl.ds(pl.multiple_of(qt * TQ, TQ), TQ)
        return gs, jnp.where(row // 16 == h % 8, qT_s[gs, qs], jnp.zeros((), bf))

    NT_ = H * NQ
    NL = TQ // TL

    def hq(i, j):
        hs = pl.ds(pl.multiple_of((i // NQ) * DH, DH), DH)
        qs = pl.ds(pl.multiple_of((i % NQ) * TQ + j * TL, TL), TL)
        return hs, qs

    def att_body(jj, bad):
        items = [(u, c) for u in range(U) for c in range(NC)]
        ctx = {}

        def stage_a(u, c):
            if c == 0:
                ctx[u] = dict(q=getq(jj * U + u), mb=[None] * NL, lo=[None] * NL, s={})
            t = ctx[u]
            gs, qm = t['q']
            for j in range(NL):
                s = jnp.dot(k_s[c * CK:(c + 1) * CK, gs], qm[:, j * TL:(j + 1) * TL],
                            preferred_element_type=f32)
                if c == 0:
                    t['mb'][j] = jnp.broadcast_to(jnp.max(s[:16], axis=0, keepdims=True), (8, TL))
                t['s'][c, j] = s

        def stage_b(u, c, bad):
            t = ctx[u]
            for j in range(NL):
                hs, qs = hq(jj * U + u, j)
                p = jnp.exp2(t['s'].pop((c, j)).reshape(CK // 8, 8, TL) - t['mb'][j][None])
                lc = jnp.sum(p, axis=0)
                oc = jnp.dot(vT_s[hs, c * CK:(c + 1) * CK], p.reshape(CK, TL).astype(bf),
                             preferred_element_type=f32)
                if c > 0:
                    lc, oc = t['lo'][j][0] + lc, t['lo'][j][1] + oc
                t['lo'][j] = (lc, oc)
                if c == NC - 1:
                    l = jnp.sum(lc, axis=0, keepdims=True)
                    oT_s[hs, qs] = oc * (1.0 / l)
                    az = jnp.abs(oc)
                    z = jnp.maximum(jnp.maximum(az[:8], az[8:]), lc)
                    bad = jnp.where(z < BIG, bad, 1.0)
            return bad

        for n in range(len(items) + SK):
            if n < len(items):
                stage_a(*items[n])
            if n >= SK:
                bad = stage_b(*items[n - SK], bad)
        return bad
    bad = jax.lax.fori_loop(0, NT_ // U, att_body, jnp.zeros((8, TL), f32))

    @pl.when(jnp.max(bad) > 0.0)
    def _():
        def tile(i, carry):
            gs, qm = getq(i)
            hs = pl.ds(pl.multiple_of((i // NQ) * DH, DH), DH)
            qs = pl.ds(pl.multiple_of((i % NQ) * TQ, TQ), TQ)

            def sc(c):
                r = pl.ds(pl.multiple_of(c * CK, CK), CK)
                return r, jnp.dot(k_s[r, gs], qm, preferred_element_type=f32)

            m = jax.lax.fori_loop(
                0, NC, lambda c, m: jnp.maximum(m, jnp.max(sc(c)[1], axis=0, keepdims=True)),
                jnp.full((1, TQ), -jnp.inf, f32))

            def acc(c, lo):
                r, s = sc(c)
                p = jnp.exp2(s - m)
                return (lo[0] + jnp.sum(p, axis=0, keepdims=True),
                        lo[1] + jnp.dot(vT_s[hs, r], p.astype(bf), preferred_element_type=f32))
            l, o = jax.lax.fori_loop(0, NC, acc, (jnp.zeros((1, TQ), f32), jnp.zeros((DH, TQ), f32)))
            oT_s[hs, qs] = o * (1.0 / l)
            return carry
        jax.lax.fori_loop(0, NT_, tile, 0)

    for cp in cps[1:]:
        cp.wait()

    def ffn_body(i, c):
        r = pl.ds(pl.multiple_of(i * TM, TM), TM)
        xn = xn_s[r, :]
        g = jnp.dot(xn, wg_ref[...], preferred_element_type=f32)
        u = jnp.dot(xn, wu_ref[...], preferred_element_type=f32)
        hh = (g * jax.nn.sigmoid(g) * u).astype(bf)
        y = jnp.dot(hh, wd_ref[...], preferred_element_type=f32)
        o = oT_s[:, r].T.astype(bf)
        a = jnp.dot(o, wo_ref[...], preferred_element_type=f32)
        o_ref[r, :] = (x_ref[r, :].astype(f32) + a + y).astype(o_ref.dtype)
        ocp(i).start()
        return c
    jax.lax.fori_loop(0, S // TM, ffn_body, 0)
    for i in range(NB):
        ocp(i).wait()


@jax.jit
def pallas_parallel_sum__mha_block__swiglu_ffn__prompt_kernel(
    A_x, A_wqkv, A_wo, B_x, B_w_gate, B_w_up, B_w_down):
    x = A_x.reshape(S, D)
    out = pl.pallas_call(
        _kernel,
        out_shape=jax.ShapeDtypeStruct((S, D), A_x.dtype),
        in_specs=[pl.BlockSpec(memory_space=pl.ANY)] * 6,
        out_specs=pl.BlockSpec(memory_space=pl.ANY),
        scratch_shapes=[
            pltpu.VMEM((S, D), bf), pltpu.VMEM((D, 3 * D), bf), pltpu.VMEM((D, D), bf),
            pltpu.VMEM((D, F), bf), pltpu.VMEM((D, F), bf), pltpu.VMEM((F, D), bf),
            pltpu.VMEM((S, D), A_x.dtype), pltpu.SemaphoreType.DMA((5 + 2 * (S // TM),)),
            pltpu.VMEM((S, D), bf), pltpu.VMEM((D, S), bf), pltpu.VMEM((S, D), bf),
            pltpu.VMEM((D, S), bf), pltpu.VMEM((D, S), f32), pltpu.VMEM((2, D, D), bf),
        ],
        compiler_params=pltpu.CompilerParams(vmem_limit_bytes=100 * 1024 * 1024),
    )(x, A_wqkv, A_wo, B_w_gate, B_w_up, B_w_down)
    return out.reshape(A_x.shape)
```
